```python
import os as _os
_os.environ.setdefault('JAX_PLATFORMS', 'cpu')
import jax
import jax.numpy as jnp

def _softmax(x, axis=-1):
    return jax.nn.softmax(x, axis=axis)

def _gelu(x):
    return jax.nn.gelu(x, approximate=True)

def _silu(x):
    return jax.nn.silu(x)

def _sigmoid(x):
    return jax.nn.sigmoid(x)

def _layernorm(x, axis=-1, eps=1e-05):
    m = jnp.mean(x, axis=axis, keepdims=True)
    v = jnp.var(x, axis=axis, keepdims=True)
    return (x - m) / jnp.sqrt(v + eps)

def _scatter_add(tgt, idx, src, axis=0):
    return tgt.at[idx].add(src)

def _segment_sum(src, seg, n):
    return jax.ops.segment_sum(src, seg, n)

class _Rng:

    def __init__(self, key):
        self._k = key

    def _next(self):
        self._k, sub = jax.random.split(self._k)
        return sub

    def normal(self, shape):
        return jax.random.normal(self._next(), shape, dtype=jnp.bfloat16)

    def randint(self, lo, hi, shape):
        return jax.random.randint(self._next(), shape, lo, hi, dtype=jnp.int32)

    def uniform(self, shape, lo=0.0, hi=1.0):
        return jax.random.uniform(self._next(), shape, jnp.bfloat16, lo, hi)

    def permutation(self, n):
        return jax.random.permutation(self._next(), n)
kernel_name = 'standalone__conformer_conv_module__speech'

def setup_inputs():
    _rng = _Rng(jax.random.key(int.from_bytes(__import__("os").urandom(4), "little")))
    _w = lambda a: (lambda t: t.astype(jnp.bfloat16) if jnp.issubdtype(t.dtype, jnp.floating) else t)(jnp.asarray(a))
    B, T, D, K = (2, 4000, 512, 15)
    return {'x': _w((lambda *s: _rng.normal(s) * 0.2)(B, T, D)), 'w_pw1': _w((lambda *s: _rng.normal(s) * 0.2)(D, 2 * D)), 'dw': _w((lambda *s: _rng.normal(s) * 0.05)(K, D)), 'w_pw2': _w((lambda *s: _rng.normal(s) * 0.05)(D, D))}

def reference(x, w_pw1, dw, w_pw2):
    B, T, D = x.shape
    K = dw.shape[0]
    h = x @ w_pw1
    a, b = (h[..., :D].copy(), h[..., D:].copy())
    h = a * _sigmoid(b)
    pad = K // 2
    hp = jnp.pad(h, ((0, 0), (pad, pad), (0, 0)))
    out = jnp.zeros_like(h)
    for i in range(K):
        out = out + hp[:, i:i + T, :] * dw[i][None, None, :]
    return _silu(out) @ w_pw2
```

```python
import functools
import jax
import jax.numpy as jnp
from jax import lax
import jax.experimental.pallas as pl
import jax.experimental.pallas.tpu as pltpu

F32 = jnp.float32
BF16 = jnp.bfloat16
I32 = jnp.int32
U32 = jnp.uint32

def make(M=400, AHEAD=2, lead=150, tail=12, gate='sel', gn=1, pk='man', rep=1, flags=None):
    B, T, D, K = 2, 4000, 512, 15
    NC = D // 128
    nb = T // M
    n = B * nb
    R = M // 16
    L = M // 8
    assert n % 2 == 0 and L % 2 == 0
    if flags: flags = {k: True for k in flags.split('+')}

    def kernel(x_hbm, w1_hbm, dw_hbm, w2_hbm, o_hbm,
               xs, w1s, w2s, dwr, dws, hA, hB, carry, gA, gB, os_, xsem, wsem, osem):
        def x_copies(j, first=False, last=False):
            if first:
                t0, sz = 0, M + 8
            elif last:
                t0, sz = j * M + 8, M - 8
            else:
                t0, sz = pl.multiple_of(j * M + 8, 8), M
            return [pltpu.make_async_copy(
                x_hbm.at[pl.ds(t0, sz), pl.ds(c * 128, 128)],
                xs.at[c, pl.ds(t0 + 8, sz), :], xsem.at[j]) for c in range(NC)]

        def o_copies(j):
            t0 = pl.multiple_of(j * M, 16)
            return [pltpu.make_async_copy(
                os_.at[c, pl.ds(t0, M), :],
                o_hbm.at[pl.ds(t0, M), pl.ds(c * 128, 128)], osem.at[j]) for c in range(NC)]

        def start(cs):
            for cp in cs: cp.start()
        def wait(cs):
            for cp in cs: cp.wait()
        def xc(j):
            return x_copies(j, j == 0, j == n - 1)

        cw1 = [pltpu.make_async_copy(w1_hbm.at[:, pl.ds(t * 128, 128)], w1s.at[t], wsem.at[0]) for t in range(2 * NC)]
        cw2 = [pltpu.make_async_copy(w2_hbm.at[:, pl.ds(t * 128, 128)], w2s.at[t], wsem.at[1]) for t in range(NC)]
        cdw = pltpu.make_async_copy(dw_hbm, dwr, wsem.at[2])
        start(xc(0))
        start(cw1)
        for c in range(NC):
            xs[c, 0:8, :] = jnp.zeros((8, 128), BF16)
            xs[c, pl.ds(n * M + 8, 8), :] = jnp.zeros((8, 128), BF16)

        xsi = xs.bitcast(I32)
        w1i = w1s.bitcast(I32)
        w2i = w2s.bitcast(I32)

        def mm(lhs, wref, t):
            return jnp.dot(lhs, pltpu.bitcast(wref[t], BF16), preferred_element_type=F32)

        def put_h(j, c, h, v, first):
            if first:
                h[c, 0:8, :] = jnp.zeros((8, 128), F32)
                h[c, 8:M + 16, :] = v[8:]
                carry[c] = v[M:]
            else:
                last = j % nb == nb - 1
                h[c, 0:16, :] = carry[c]
                h[c, 16:M + 8, :] = v[:M - 8]
                h[c, M + 8:M + 16, :] = jnp.where(last, 0.0, v[M - 8:])
                carry[c, 0:8, :] = jnp.where(last, 0.0, v[M - 16:M - 8])
                carry[c, 8:16, :] = v[M - 8:]

        def pack2(lo, hi):
            if pk == 'man':
                lo = pltpu.bitcast(lo.astype(BF16).astype(F32), U32) >> 16
                hi = pltpu.bitcast(hi.astype(BF16).astype(F32), U32)
                return pltpu.bitcast(lo | hi, I32)
            return pltpu.bitcast(pltpu.pack_elementwise([lo, hi], packed_dtype=BF16), I32)

        def conv_gen(h, g, never):
            work = 0
            for c in range(NC):
                w = None
                acc = {}
                done = {}
                for m0 in range(0, L + K - 1, gn):
                    gv = yield work
                    if gv is not None and gate == 'st':
                        a0 = (m0 + 1) // 8 * 8
                        pltpu.store(h.at[c, pl.ds(a0, 8), :], gv, mask=never)
                    if w is None:
                        w = [dws[c, k] for k in range(K)]
                    for m in range(m0, min(m0 + gn, L + K - 1)):
                        hv = h[c, pl.ds(m + 1, 8, stride=L), :]
                        if gv is not None and gate == 'sel':
                            hv = jnp.where(never, gv, hv)
                        for k in range(K):
                            jj = m - k
                            if 0 <= jj < L:
                                t = hv * w[k]
                                acc[jj] = t if k == 0 else acc[jj] + t
                                work += 2
                        jj = m - (K - 1)
                        if jj >= 0:
                            z = acc.pop(jj)
                            done[jj] = z * jnp.tanh(z) + z
                            work += 4
                            if jj % 2 == 1:
                                g[c, pl.ds(jj // 2, 8, stride=L // 2), :] = pack2(done.pop(jj - 1), done.pop(jj))
            yield None
        total_work = NC * L * (2 * K + 4)

        def step(j, par, do1=True, do2=True, do3=True):
            first = isinstance(j, int) and j == 0
            h1, h2 = (hA, hB) if par == 0 else (hB, hA)
            g2, g3 = (gB, gA) if par == 0 else (gA, gB)
            ngroups = R * NC * (2 * do1 + do3)
            st = dict(g=0, w=None)
            if do2:
                never = (w2i[0, 0:8, :] | 1) == 0
                gen = conv_gen(h2, g2, never)
                st['w'] = next(gen)
                while st['w'] is not None and st['w'] < lead:
                    st['w'] = gen.send(None)
            def release(res):
                for r in range(2 * R):
                    while st['w'] is not None and (st['w'] - lead) * 2 * (ngroups - tail) <= st['g'] * (total_work - lead):
                        st['w'] = gen.send(res[8 * r:8 * r + 8])
                    st['g'] += 1
            def ldx():
                if first:
                    return jnp.concatenate([pltpu.bitcast(xsi[k, 0:M // 2 + 8, :], BF16) for k in range(NC)], axis=1)
                p0 = pl.multiple_of(j * (M // 2) + 8, 8)
                return jnp.concatenate([pltpu.bitcast(xsi[k, pl.ds(p0, M // 2), :], BF16) for k in range(NC)], axis=1)
            for c in range(NC):
                if do1:
                    a = mm(ldx(), w1i, c)
                    release(a)
                    b = mm(ldx(), w1i, NC + c)
                    release(b)
                    put_h(j, c, h1, a * jnp.tanh(b * 0.5) + a, first)
                if do3:
                    gv = jnp.concatenate([pltpu.bitcast(g3[cc], BF16) for cc in range(NC)], axis=1)
                    o = mm(gv, w2i, c)
                    release(o)
                    os_[c, pl.ds(pl.multiple_of((j - 2) * M, 16), M), :] = o.astype(BF16)
            assert st['w'] is None

        wait(xc(0))
        wait(cw1)
        start(xc(1))
        cdw.start()
        start(cw2)
        start(xc(2))
        start(xc(3))
        step(0, 0, True, False, False)
        cdw.wait()
        wait(cw2)
        wait(xc(1))
        dwv = dwr[...].astype(F32) * 0.25
        for c in range(NC):
            for k in range(K):
                dws[c, k] = jnp.broadcast_to(dwv[k:k + 1, c * 128:(c + 1) * 128], (8, 128))
        step(1, 1, True, True, False)
        start(xc(n - 1))
        def body(it, _):
            j = 2 * it
            wait(x_copies(j))
            @pl.when(j + 1 < n - 1)
            def _():
                wait(x_copies(j + 1))
                start(x_copies(j + 2))
            @pl.when(j + 3 < n - 1)
            def _():
                start(x_copies(j + 3))
            @pl.when(j + 1 == n - 1)
            def _():
                wait(xc(n - 1))
            step(j, 0)
            start(o_copies(j - 2))
            step(j + 1, 1)
            start(o_copies(j - 1))
            return 0
        lax.fori_loop(1, n // 2, body, 0)
        if rep > 1:
            def body2(it, _):
                step(2 + 2 * (it % 4), 0)
                step(3 + 2 * (it % 4), 1)
                return 0
            lax.fori_loop(0, rep - 1, body2, 0)
        step(n, 0, False, True, True)
        start(o_copies(n - 2))
        step(n + 1, 1, False, False, True)
        start(o_copies(n - 1))
        for j in range(n):
            wait(o_copies(j))

    def f(x, w_pw1, dw, w_pw2):
        out = pl.pallas_call(
            kernel,
            in_specs=[pl.BlockSpec(memory_space=pl.ANY)] * 4,
            out_specs=pl.BlockSpec(memory_space=pl.ANY),
            out_shape=jax.ShapeDtypeStruct((B * T, D), x.dtype),
            scratch_shapes=[
                pltpu.VMEM((NC, n * M + 16, 128), BF16),
                pltpu.VMEM((2 * NC, D, 128), BF16),
                pltpu.VMEM((NC, D, 128), BF16),
                pltpu.VMEM((K, D), BF16),
                pltpu.VMEM((NC, K, 8, 128), F32),
                pltpu.VMEM((NC, M + 16, 128), F32),
                pltpu.VMEM((NC, M + 16, 128), F32),
                pltpu.VMEM((NC, 16, 128), F32),
                pltpu.VMEM((NC, M // 2, 128), I32),
                pltpu.VMEM((NC, M // 2, 128), I32),
                pltpu.VMEM((NC, n * M, 128), BF16),
                pltpu.SemaphoreType.DMA((n,)),
                pltpu.SemaphoreType.DMA((3,)),
                pltpu.SemaphoreType.DMA((n,)),
            ],
            compiler_params=pltpu.CompilerParams(vmem_limit_bytes=100 * 2**20, flags=flags),
        )(x.reshape(B * T, D), w_pw1, dw, w_pw2)
        return out.reshape(B, T, D)
    return f


@jax.jit
def pallas_standalone__conformer_conv_module__speech_kernel(x, w_pw1, dw, w_pw2):
    return make()(x, w_pw1, dw, w_pw2)
```

```python
import jax
import jax.numpy as jnp
from jax import lax
import jax.experimental.pallas as pl
import jax.experimental.pallas.tpu as pltpu

_LANES = 128
_M = 400
_L = _M // 8
_UNROLL = 2
_HALO = 8

_START_TILES = (0, 1, 3, 6, 16)
_START_WORK = (0.0, 0.25, 1.6, 6.0)
_LEAD = 18
_TAIL = 12
_LAST_ROWS = (256, 128, 16)


def _sigmoid(v):
    d = 1.0 + jnp.exp2(jnp.minimum(v * -1.4426950408889634, 126.0))
    r = pltpu.reciprocal(d, approx=True)
    return r * (2.0 - d * r)


def _pack_row_pairs(lo, hi):
    lo = pltpu.bitcast(lo.astype(jnp.bfloat16).astype(jnp.float32), jnp.uint32)
    hi = pltpu.bitcast(hi.astype(jnp.bfloat16).astype(jnp.float32), jnp.uint32)
    return pltpu.bitcast((lo >> 16) | hi, jnp.int32)


def _load_bf16(raw, words, first_use):
    if not first_use:
        return pltpu.bitcast(words[...], jnp.bfloat16)
    v = raw[...]
    words[...] = pltpu.bitcast(v, jnp.int32)
    return v


def _start(copies, priority=0):
    for cp in copies:
        cp.start(priority=priority)


def _wait(copies):
    for cp in copies:
        cp.wait()


class _Fir:
    def __init__(self, h, taps, jobs, h_tag):
        self.h, self.taps, self.jobs, self.h_tag = h, taps, list(jobs), h_tag
        self.ntaps = taps.shape[1]
        self.job_work = _L * (2 * self.ntaps + 8)
        self.work = self.budget = 0
        self.m = 0

    def pending(self, tag, c=None):
        return any(t == tag and c in (None, jc) for t, jc, _ in self.jobs)

    def advance(self, goal, fraction, never=None, gate=None):
        self.budget += (goal * self.job_work - self.budget) * fraction
        while self.jobs and self.work < self.budget:
            tag, c, _ = self.jobs[0]
            if self.h_tag[c] != tag:
                self.budget = self.work
                break
            self._step(never, gate)

    def _step(self, never, gate):
        _, c, g = self.jobs[0]
        m, ntaps = self.m, self.ntaps
        if m == 0:
            self.w = [self.taps[c, k] for k in range(ntaps)]
            self.acc = {}
        hv = self.h[c, pl.ds(m + _HALO - ntaps // 2, 8, stride=_L), :]
        if gate is not None:
            hv = jnp.where(never, gate, hv)
        for k in range(ntaps):
            if 0 <= m - k < _L:
                t = hv * self.w[k]
                self.acc[m - k] = t if k == 0 else self.acc[m - k] + t
                self.work += 2
        last = m - (ntaps - 1)
        if last >= 0:
            z = self.acc.pop(last)
            y = z * _sigmoid(z)
            self.work += 8
            if last % 2 == 0:
                self.even = y
            else:
                g[c, pl.ds(last // 2, 8, stride=_L // 2), :] = _pack_row_pairs(self.even, y)
        self.m += 1
        if last == _L - 1:
            self.m = 0
            self.jobs.pop(0)


def _kernel(x_hbm, w1_hbm, dw_hbm, w2_hbm, o_hbm,
            xs, w1s, w2s, x_words, w1_words, dw_raw,
            taps, h, carry, g0, g1, outs, xsem, wsem, osem,
            *, chunks_per_batch):
    n, nc = outs.shape[:2]
    ntaps = dw_raw.shape[0]
    n_iter = (n - 2) // _UNROLL
    gbuf = (g0, g1)
    zeros = jnp.zeros((_HALO, _LANES), jnp.float32)

    def cols(c):
        return pl.ds(c * _LANES, _LANES)

    def x_copy(j, sem):
        if isinstance(j, int) and j == 0:
            src, rows, dst = 0, _M + _HALO, _HALO
        elif isinstance(j, int) and j == n - 1:
            src, rows, dst = j * _M + _HALO, _M - _HALO, 0
        else:
            src, rows, dst = pl.multiple_of(j * _M + _HALO, _HALO), _M, 0
        return pltpu.make_async_copy(x_hbm.at[pl.ds(src, rows), :],
                                     xs.at[j, pl.ds(dst, rows), :], xsem.at[sem])

    def x_copies_for_iter(i):
        return [x_copy(2 + _UNROLL * i + u, 0) for u in range(_UNROLL)]

    def matmul(lhs_blocks, rhs):
        return jnp.dot(jnp.concatenate(lhs_blocks, axis=1), rhs,
                       preferred_element_type=jnp.float32)

    def store_glu(j, c, v):
        if isinstance(j, int) and j == 0:
            h[c, 0:_HALO, :] = zeros
            h[c, _HALO:_M + 2 * _HALO, :] = v[_HALO:]
            carry[c] = v[_M:]
            return
        ends_batch = j == chunks_per_batch - 1
        for b in range(2, n // chunks_per_batch + 1):
            ends_batch = ends_batch | (j == b * chunks_per_batch - 1)
        before, after = v[_M - 2 * _HALO:_M - _HALO], v[_M - _HALO:]
        h[c, 0:2 * _HALO, :] = carry[c]
        h[c, 2 * _HALO:_M + _HALO, :] = v[:_M - _HALO]
        h[c, _M + _HALO:_M + 2 * _HALO, :] = jnp.where(ends_batch, zeros, after)
        carry[c, 0:_HALO, :] = jnp.where(ends_batch, zeros, before)
        carry[c, _HALO:2 * _HALO, :] = after

    def store_out(j, c, v):
        final = isinstance(j, int) and j == n - 1 and c == nc - 1
        r0 = 0
        for rows in _LAST_ROWS if final else (_M,):
            outs[j, c, r0:r0 + rows, :] = v[r0:r0 + rows].astype(outs.dtype)
            dst = pl.multiple_of(j * _M + r0, 16)
            pltpu.make_async_copy(outs.at[j, c, pl.ds(r0, rows), :],
                                  o_hbm.at[pl.ds(dst, rows), cols(c)], osem.at[0]).start()
            r0 += rows

    def pw1(tag, j):
        return [(kind, tag, j, c) for c in range(nc) for kind in ("gate", "value")]

    def pw2(tag, j):
        return [("out", tag, j, c) for c in range(nc)]

    def run(tiles, fir, goal, slots, glu_gate):
        never = (pltpu.bitcast(taps[0, 0], jnp.int32) | 1) == 0
        fir.advance(goal, _LEAD / (slots + _LEAD))
        for kind, tag, j, c in tiles:
            if kind == "out":
                assert not fir.pending(tag)
                v = matmul([pltpu.bitcast(gbuf[tag % 2][k, 0:_M // 2, :], jnp.bfloat16)
                            for k in range(nc)], w2s[:, cols(c)])
            else:
                first_chunk = isinstance(j, int) and j == 0
                rows = _M + (2 * _HALO if first_chunk else 0)
                t = nc + c if kind == "gate" else c
                v = matmul([_load_bf16(xs.at[j, pl.ds(0, rows), cols(k)],
                                       x_words.at[k, pl.ds(0, rows // 2), :], t == nc)
                            for k in range(nc)],
                           _load_bf16(w1s.at[t], w1_words.at[t], first_chunk))
            for r in range(v.shape[0] - _M, v.shape[0], 8):
                fir.advance(goal, 1 / max(slots, 1), never, v[r:r + 8])
                slots -= 1
            if kind == "gate":
                glu_gate.append(_sigmoid(v))
            elif kind == "value":
                assert not fir.pending(tag - 1, c)
                store_glu(j, c, v * glu_gate.pop())
                fir.h_tag[c] = tag
            else:
                store_out(j, c, v)

    def conv_jobs(tag, columns):
        return [(tag, c, gbuf[tag % 2]) for c in columns]

    early, late = range(nc // 2), range(nc // 2, nc)

    first_tiles = pw1(0, 0) + pw1(1, 1)
    stretches = [first_tiles[a:b] for a, b in zip(_START_TILES, _START_TILES[1:])]
    groups = []
    for q, tiles in enumerate(stretches):
        blocks = [nc + c if kind == "gate" else c for kind, tag, _, c in tiles if tag == 0]
        groups.append([pltpu.make_async_copy(w1_hbm.at[:, cols(t)], w1s.at[t], wsem.at[2 + q])
                       for t in blocks])
    groups[0].append(x_copy(0, 0))
    groups[-1].append(x_copy(1, 1))
    w2_copy = pltpu.make_async_copy(w2_hbm, w2s, wsem.at[0])
    groups += [[w2_copy] + x_copies_for_iter(0), [], []]
    dw_copy = pltpu.make_async_copy(dw_hbm, dw_raw, wsem.at[1])

    xs[0, 0:_HALO, :] = jnp.zeros((_HALO, nc * _LANES), xs.dtype)
    xs[n - 1, _M - _HALO:_M, :] = jnp.zeros((_HALO, nc * _LANES), xs.dtype)
    dw_copy.start()
    _start(groups[0])
    _start(groups[1], priority=1)
    for c in range(nc):
        h[c, _M + 2 * _HALO:, :] = jnp.zeros((h.shape[1] - _M - 2 * _HALO, _LANES), h.dtype)
    dw_copy.wait()
    _start(groups[2], priority=1)
    dw = dw_raw[...].astype(jnp.float32)
    for c in range(nc):
        for k in range(ntaps):
            taps[c, k] = jnp.broadcast_to(dw[k:k + 1, c * _LANES:(c + 1) * _LANES], (8, _LANES))

    fir = _Fir(h, taps, conv_jobs(0, range(nc)) + conv_jobs(1, early), [None] * nc)
    glu_gate = []
    for q, tiles in enumerate(stretches):
        _wait(groups[q])
        _start(groups[q + 3], priority=1)
        run(tiles, fir, _START_WORK[q], len(tiles) * _L - _TAIL, glu_gate)
    assert not fir.jobs
    w2_copy.wait()

    def body(i, _):
        @pl.when(i < n_iter - 1)
        def _():
            _wait(x_copies_for_iter(i))

        @pl.when(i == n_iter - 1)
        def _():
            _wait(x_copies_for_iter(n_iter - 1))

        @pl.when(i + 1 < n_iter - 1)
        def _():
            _start(x_copies_for_iter(i + 1))

        @pl.when(i + 1 == n_iter - 1)
        def _():
            _start(x_copies_for_iter(n_iter - 1))

        tiles, jobs = [], []
        for u in range(_UNROLL):
            j = 2 + _UNROLL * i + u
            tiles += pw2(u - 2, j - 2) + pw1(u, j)
            jobs += conv_jobs(u - 1, late) + conv_jobs(u, early)
        fir = _Fir(h, taps, jobs, [-1] * nc)
        run(tiles, fir, len(jobs), len(tiles) * _L - _TAIL, [])
        assert not fir.jobs

    lax.fori_loop(0, n_iter, body, None)

    fir = _Fir(h, taps, conv_jobs(1, late), [1] * nc)
    run(pw2(0, n - 2) + pw2(1, n - 1), fir, len(late), nc * _L - 2 * _TAIL, [])
    pltpu.make_async_copy(o_hbm, o_hbm, osem.at[0]).wait()


@jax.jit
def pallas_standalone__conformer_conv_module__speech_kernel(
    x: jax.Array,
    w_pw1: jax.Array,
    dw: jax.Array,
    w_pw2: jax.Array,
):
    B, T, D = x.shape
    K = dw.shape[0]
    nc = D // _LANES
    n = B * T // _M
    assert x.dtype == jnp.bfloat16 and nc == 4 and D == nc * _LANES
    assert T % _M == 0 and T > _M and (n - 2) % _UNROLL == 0 and _UNROLL % 2 == 0
    assert K % 2 == 1 and K // 2 <= _HALO and sum(_LAST_ROWS) == _M

    def kernel(*refs):
        _kernel(*refs, chunks_per_batch=T // _M)

    g_shape = (nc, _M // 2 + 24, _LANES)
    out = pl.pallas_call(
        kernel,
        in_specs=[pl.BlockSpec(memory_space=pl.ANY)] * 4,
        out_specs=pl.BlockSpec(memory_space=pl.ANY),
        out_shape=jax.ShapeDtypeStruct((B * T, D), x.dtype),
        scratch_shapes=[
            pltpu.VMEM((n, _M + 2 * _HALO, D), x.dtype),
            pltpu.VMEM((2 * nc, D, _LANES), w_pw1.dtype),
            pltpu.VMEM((D, D), w_pw2.dtype),
            pltpu.VMEM((nc, _M // 2 + _HALO, _LANES), jnp.int32),
            pltpu.VMEM((2 * nc, D // 2, _LANES), jnp.int32),
            pltpu.VMEM((K, D), dw.dtype),
            pltpu.VMEM((nc, K, 8, _LANES), jnp.float32),
            pltpu.VMEM((nc, _M + 72, _LANES), jnp.float32),
            pltpu.VMEM((nc, 2 * _HALO, _LANES), jnp.float32),
            pltpu.VMEM(g_shape, jnp.int32),
            pltpu.VMEM(g_shape, jnp.int32),
            pltpu.VMEM((n, nc, _M, _LANES), x.dtype),
            pltpu.SemaphoreType.DMA((2,)),
            pltpu.SemaphoreType.DMA((len(_START_TILES) + 1,)),
            pltpu.SemaphoreType.DMA((1,)),
        ],
        compiler_params=pltpu.CompilerParams(
            vmem_limit_bytes=64 * 1024 * 1024, disable_bounds_checks=True),
    )(x.reshape(B * T, D), w_pw1, dw, w_pw2)
    return out.reshape(B, T, D)
```
